```python
import jax
import jax.numpy as jnp

def _softmax(x, axis=-1):
    return jax.nn.softmax(x, axis=axis)
def _gelu(x):
    return jax.nn.gelu(x, approximate=True)
def _silu(x):
    return jax.nn.silu(x)
def _sigmoid(x):
    return jax.nn.sigmoid(x)
def _layernorm(x, axis=-1, eps=1e-5):
    m = jnp.mean(x, axis=axis, keepdims=True)
    v = jnp.var(x, axis=axis, keepdims=True)
    return (x - m) / jnp.sqrt(v + eps)
def _scatter_add(tgt, idx, src, axis=0):
    return tgt.at[idx].add(src)
def _segment_sum(src, seg, n):
    return jax.ops.segment_sum(src, seg, n)
class _Rng:
    def __init__(self, key):
        self._k = key
    def _next(self):
        self._k, sub = jax.random.split(self._k)
        return sub
    def normal(self, shape):
        return jax.random.normal(self._next(), shape, dtype=jnp.bfloat16)
    def randint(self, lo, hi, shape):
        return jax.random.randint(self._next(), shape, lo, hi, dtype=jnp.int32)
    def uniform(self, shape, lo=0.0, hi=1.0):
        return jax.random.uniform(self._next(), shape, jnp.bfloat16, lo, hi)
    def permutation(self, n):
        return jax.random.permutation(self._next(), n)


kernel_name = 'interleave_layers__sliding_block_cached__mixer_s_mlp__decode'

def setup_inputs():
    _rng = _Rng(jax.random.key(int.from_bytes(__import__("os").urandom(4), "little")))
    _w = (lambda a: (lambda t: t.astype(jnp.bfloat16) if jnp.issubdtype(t.dtype, jnp.floating) else t)(jnp.asarray(a)))
    def _A_setup():
        B, Sq, D = 1, 1, 640
        Hq, Hkv, Sk, Dh = 32, 32, 32768, 192
        assert Hq % Hkv == 0, (Hq, Hkv)
        return {
            "x": _w((lambda *s: _rng.normal(s) * 0.05)(B, Sq, D)),
            "k_cache": _w((lambda *s: _rng.normal(s) * 0.05)(B, Hkv, Sk, Dh)),
            "v_cache": _w((lambda *s: _rng.normal(s) * 0.05)(B, Hkv, Sk, Dh)),
            "wq": _w((lambda *s: _rng.normal(s) * 0.05)(D, Hq * Dh) * (D ** -0.5)),
            "wo": _w((lambda *s: _rng.normal(s) * 0.05)(Hq * Dh, D) * ((Hq * Dh) ** -0.5)),
        }
    _A_in = _A_setup()

    def _B_setup():
        B, S, D, F = 1, 1, 640, 1536
        return {
            "x":  _w((lambda *s: _rng.normal(s) * 0.05)(B, S, D)),
            "w1": _w((lambda *s: _rng.normal(s) * 0.05)(D, D) * (D ** -0.5)),
            "w2": _w((lambda *s: _rng.normal(s) * 0.05)(D, D) * (D ** -0.5)),
            "w3": _w((lambda *s: _rng.normal(s) * 0.05)(D, F) * (D ** -0.5)),
            "w4": _w((lambda *s: _rng.normal(s) * 0.05)(F, D) * (F ** -0.5)),
        }
    _B_in = _B_setup()

    return {
        "A_x": _A_in["x"],
        "A_k_cache": _A_in["k_cache"],
        "A_v_cache": _A_in["v_cache"],
        "A_wq": _A_in["wq"],
        "A_wo": _A_in["wo"],
        "B_x": _B_in["x"],
        "B_w1": _B_in["w1"],
        "B_w2": _B_in["w2"],
        "B_w3": _B_in["w3"],
        "B_w4": _B_in["w4"],
    }

def reference(A_x, A_k_cache, A_v_cache, A_wq, A_wo, B_x, B_w1, B_w2, B_w3, B_w4):
    def _A_ref(x, k_cache, v_cache, wq, wo):
        B, Sq, D = x.shape
        Hq, Dh = 32, 192
        Hkv, Sk = k_cache.shape[1], k_cache.shape[2]
        W = min(4096, max(256, Sk // 4))
        rep = Hq // Hkv
        q = (lambda x, *d: x.transpose(*d))((x @ wq).reshape(B, Sq, Hq, Dh), 0, 2, 1, 3)
        k = jnp.repeat(k_cache[:, :, Sk - W:, :], rep, axis=1)
        v = jnp.repeat(v_cache[:, :, Sk - W:, :], rep, axis=1)
        scores = jnp.einsum("bhqd,bhkd->bhqk", q, k) * (Dh ** -0.5)
        p = _softmax(scores, axis=-1)
        o = jnp.einsum("bhqk,bhkd->bhqd", p, v)
        return (lambda x, *d: x.transpose(*d))(o, 0, 2, 1, 3).reshape(B, Sq, Hq * Dh) @ wo

    def _B_ref(x, w1, w2, w3, w4):
        B, S, D = x.shape
        h = _gelu(_layernorm(x, axis=-1) @ w1)
        c = D // 4
        g0 = jnp.pad(h[:, :, 0*c:1*c], ((0, 0), (1, 0), (0, 0)))[:, :S, :]
        g1 = jnp.pad(h[:, :, 1*c:2*c], ((0, 0), (0, 1), (0, 0)))[:, 1:, :]
        g2 = jnp.pad(h[:, :, 2*c:3*c], ((0, 0), (2, 0), (0, 0)))[:, :S, :]
        g3 = jnp.pad(h[:, :, 3*c:   ], ((0, 0), (0, 2), (0, 0)))[:, 2:, :]
        hs = jnp.concatenate([g0, g1, g2, g3], axis=-1) @ w2
        x1 = x + hs
        h2 = _gelu(_layernorm(x1, axis=-1) @ w3) @ w4
        return x1 + h2

    x = A_x
    x = x + _A_ref(_layernorm(x, axis=-1), A_k_cache, A_v_cache, A_wq, A_wo)
    x = x + _B_ref(_layernorm(x, axis=-1), B_w1, B_w2, B_w3, B_w4)
    x = x + _A_ref(_layernorm(x, axis=-1), A_k_cache, A_v_cache, A_wq, A_wo)
    x = x + _B_ref(_layernorm(x, axis=-1), B_w1, B_w2, B_w3, B_w4)
    return x
```

```python
import functools

import jax
import jax.numpy as jnp
import numpy as np
from jax import lax
from jax.experimental import pallas as pl
from jax.experimental.pallas import tpu as pltpu

D = 640
NH = 32
DH = 192
SK = 32768
W = 4096
FF = 1536
NP = NH // 2
NCB = W // 128
CB0 = (SK - W) // 128
EPS = 1e-5
LOG2E = 1.4426950408889634
QSCALE = (DH ** -0.5) * LOG2E
AG = 6

_MASK_HI = np.int32(-65536)


def _tiles_k(c):
    t = jnp.transpose(c[0], (0, 2, 1)).reshape(NP, 24, 2, 8, SK // 128, 128)
    return jnp.transpose(t, (0, 1, 2, 4, 3, 5))


def _tiles_w(w):
    k, n = w.shape
    return jnp.transpose(w.reshape(k // 16, 2, 8, n // 128, 128), (0, 1, 3, 2, 4))


def _as_bf16(words):
    n = words.shape[0]
    return pltpu.bitcast(words.reshape(n * 8, 128), jnp.bfloat16)


def _mm(a, b):
    return jnp.dot(a, b, preferred_element_type=jnp.float32)


def _layernorm(x):
    m = jnp.mean(x, axis=-1, keepdims=True)
    d = x - m
    v = jnp.mean(d * d, axis=-1, keepdims=True)
    return d * lax.rsqrt(v + EPS)


def _gelu(x):
    c = np.float32(0.7978845608028654)
    return 0.5 * x * (1.0 + jnp.tanh(c * (x + np.float32(0.044715) * (x * x * x))))


def _kernel(x_hbm, k_hbm, v_hbm, wq_hbm, wo_hbm, w3_hbm, w4_hbm, o_ref,
            xbuf, kbuf, vbuf, wqbuf, wobuf, w3buf, w4buf, lbuf, pbuf, zbuf, ibuf,
            kv_sem, w_sem):
    ki = k_hbm.bitcast(jnp.int32)
    vi = v_hbm.bitcast(jnp.int32)

    def kv_copy(t, g, b):
        src, dst = ((ki, kbuf), (vi, vbuf))[t]
        return pltpu.make_async_copy(src.at[g, :, b, pl.ds(CB0, NCB)],
                                     dst.at[g, :, :, pl.ds(4 * b, 4), :], kv_sem.at[t, g, b])

    def w_copy(i, b):
        src, dst = ((wq_hbm, wqbuf), (wo_hbm, wobuf), (w3_hbm, w3buf), (w4_hbm, w4buf))[i]
        return pltpu.make_async_copy(src.bitcast(jnp.int32).at[:, b],
                                     dst.at[:, :, pl.ds(4 * b, 4), :], w_sem.at[i, b])

    x_copy = pltpu.make_async_copy(x_hbm, xbuf, w_sem.at[4, 0])

    x_copy.start()
    for b in range(2):
        w_copy(0, b).start()
    for g in range(NP):
        for t in range(2):
            for b in range(2):
                kv_copy(t, g, b).start()
    for i in (1, 2, 3):
        for b in range(2):
            w_copy(i, b).start()

    def wait_w(i):
        for b in range(2):
            w_copy(i, b).wait()

    def wait_kv(t, g):
        for b in range(2):
            kv_copy(t, g, b).wait()

    rows = lax.broadcasted_iota(jnp.int32, (8, 128), 0)
    lanes = lax.broadcasted_iota(jnp.int32, (8, 128), 1)
    lane_lo = lanes < 64

    def make_q(y_bf, g):
        q = [_mm(y_bf, _as_bf16(wqbuf[:, 3 * g + c])) * np.float32(QSCALE) for c in range(3)]
        for r in range(4):
            ra = rows == 2 * r
            rb = rows == 2 * r + 1
            l0 = jnp.where(ra, q[0], 0.0)
            l1 = jnp.where((ra & lane_lo) | (rb & (~lane_lo)), q[1], 0.0)
            l2 = jnp.where(rb, q[2], 0.0)
            lbuf[g, r] = jnp.concatenate([l0, l1, l2], axis=1).astype(jnp.bfloat16)

    def qk(g):
        lhs = [lbuf[g, r] for r in range(4)]
        out = []
        for i in range(8):
            tot = None
            for r in range(4):
                s = _mm(lhs[r], _as_bf16(kbuf[g, :, 4 * i + r]))
                tot = s if tot is None else tot + s
            out.append(tot)
        return out

    def softmax_to(slot, sc):
        m = sc[0]
        for s in sc[1:]:
            m = jnp.maximum(m, s)
        m = jnp.max(m, axis=1, keepdims=True)
        m = jnp.broadcast_to(m, (8, 128))
        m = jnp.maximum(m, pltpu.roll(m, 2, 0))
        m = jnp.maximum(m, pltpu.roll(m, 4, 0))
        tot = None
        for i in range(8):
            p = jnp.exp2(sc[i] - m)
            pbuf[slot, i] = p
            tot = p if tot is None else tot + p
        l = jnp.broadcast_to(jnp.sum(tot, axis=1, keepdims=True), (8, 128))
        l = l + pltpu.roll(l, 2, 0)
        l = l + pltpu.roll(l, 4, 0)
        ibuf[slot] = 1.0 / l

    def pv(g, slot):
        for e in range(2):
            for a0 in range(0, 12, AG):
                acc = [[None, None] for _ in range(AG)]
                for cb in range(NCB):
                    row = 2 * (cb % 4) + e
                    p = jnp.broadcast_to(pbuf[slot, cb // 4, row:row + 1, :], (8, 128))
                    for a in range(AG):
                        w = vbuf[g, 12 * e + a0 + a, cb]
                        lo = pltpu.bitcast(w << 16, jnp.float32) * p
                        hi = pltpu.bitcast(w & _MASK_HI, jnp.float32) * p
                        A = acc[a]
                        A[0] = lo if A[0] is None else A[0] + lo
                        A[1] = hi if A[1] is None else A[1] + hi
                for a in range(AG):
                    z = pltpu.pack_elementwise(acc[a], packed_dtype=jnp.bfloat16)
                    zbuf[slot, 12 * e + a0 + a] = pltpu.bitcast(z, jnp.int32)

    ones_bf = jnp.ones((8, 128), jnp.bfloat16)

    def o_proj(g, slot, xacc):
        inv = ibuf[slot]
        inv_a = jnp.broadcast_to(inv[0:1, :], (8, 128))
        inv_b = jnp.broadcast_to(inv[1:2, :], (8, 128))
        scale = (inv_a, jnp.where(lane_lo, inv_a, inv_b), inv_b)
        o = []
        for t in range(3):
            z = _as_bf16(zbuf[slot, 8 * t:8 * t + 8])
            r = lax.dot_general(ones_bf, z, (((1,), (1,)), ((), ())),
                                preferred_element_type=jnp.float32)
            o.append(r * scale[t])
        o_bf = jnp.concatenate(o, axis=1).astype(jnp.bfloat16)
        return [xacc[c] + _mm(o_bf, _as_bf16(wobuf[pl.ds(24 * g, 24), c])) for c in range(5)]

    def attention(x, first):
        y_bf = _layernorm(x).astype(jnp.bfloat16)
        if first:
            wait_w(0)

        def q_body(g, c):
            make_q(y_bf, g)
            return c
        lax.fori_loop(0, NP, q_body, 0)

        if first:
            wait_kv(0, 0)
        softmax_to(0, qk(0))

        def body(g, xacc):
            slot = g & 1
            gn = jnp.minimum(g + 1, NP - 1)
            if first:
                @pl.when(g + 1 < NP)
                def _():
                    wait_kv(0, g + 1)
                wait_kv(1, g)
            sc = qk(gn)
            pv(g, slot)
            softmax_to(1 - slot, sc)
            return xacc

        zero = jnp.zeros((8, 128), jnp.float32)
        lax.fori_loop(0, NP, body, 0)
        return None

    x_copy.wait()
    x = jnp.broadcast_to(xbuf[0].astype(jnp.float32), (8, D))

    def attn_layer(x, first):
        y_bf = _layernorm(x).astype(jnp.bfloat16)
        if first:
            wait_w(0)

        def q_body(g, c):
            make_q(y_bf, g)
            return c
        lax.fori_loop(0, NP, q_body, 0)

        if first:
            wait_kv(0, 0)
        softmax_to(0, qk(0))

        def body(g, c):
            slot = g & 1
            gn = jnp.minimum(g + 1, NP - 1)
            if first:
                @pl.when(g + 1 < NP)
                def _():
                    wait_kv(0, g + 1)
                wait_kv(1, g)
            sc = qk(gn)
            pv(g, slot)
            ibuf_keep = ibuf[slot]
            ibuf[2 + g] = ibuf_keep
            softmax_to(1 - slot, sc)
            for a in range(24):
                zbuf[2 + g, a] = zbuf[slot, a]
            return c
        lax.fori_loop(0, NP, body, 0)

        if first:
            wait_w(1)

        def o_body(g, xacc):
            return tuple(o_proj(g, 2 + g, list(xacc)))
        zero = jnp.zeros((8, 128), jnp.float32)
        xacc = lax.fori_loop(0, NP, o_body, (zero,) * 5)
        return x + jnp.concatenate(xacc, axis=1)

    def mlp_layer(x, first):
        y = _layernorm(x)
        u_bf = _layernorm(y).astype(jnp.bfloat16)
        if first:
            wait_w(2)
        h = jnp.concatenate([_mm(u_bf, _as_bf16(w3buf[:, c])) for c in range(FF // 128)], axis=1)
        h_bf = _gelu(h).astype(jnp.bfloat16)
        if first:
            wait_w(3)
        h2 = jnp.concatenate([_mm(h_bf, _as_bf16(w4buf[:, c])) for c in range(D // 128)], axis=1)
        return x + (y + h2)

    x = attn_layer(x, True)
    x = mlp_layer(x, True)
    x = attn_layer(x, False)
    x = mlp_layer(x, False)
    o_ref[0] = x[0:1, :].astype(o_ref.dtype)


@jax.jit
def pallas_interleave_layers__sliding_block_cached__mixer_s_mlp__decode_kernel(
    A_x: jax.Array,
    A_k_cache: jax.Array,
    A_v_cache: jax.Array,
    A_wq: jax.Array,
    A_wo: jax.Array,
    B_x: jax.Array,
    B_w1: jax.Array,
    B_w2: jax.Array,
    B_w3: jax.Array,
    B_w4: jax.Array,
):
    del B_x, B_w1, B_w2
    any_spec = pl.BlockSpec(memory_space=pl.ANY)
    return pl.pallas_call(
        _kernel,
        out_shape=jax.ShapeDtypeStruct((1, 1, D), A_x.dtype),
        in_specs=[any_spec] * 7,
        out_specs=pl.BlockSpec(memory_space=pltpu.VMEM),
        scratch_shapes=[
            pltpu.VMEM((1, 1, D), jnp.bfloat16),
            pltpu.VMEM((NP, 24, NCB, 8, 128), jnp.int32),
            pltpu.VMEM((NP, 24, NCB, 8, 128), jnp.int32),
            pltpu.VMEM((D // 16, NH * DH // 128, 8, 128), jnp.int32),
            pltpu.VMEM((NH * DH // 16, D // 128, 8, 128), jnp.int32),
            pltpu.VMEM((D // 16, FF // 128, 8, 128), jnp.int32),
            pltpu.VMEM((FF // 16, D // 128, 8, 128), jnp.int32),
            pltpu.VMEM((NP, 4, 8, 384), jnp.bfloat16),
            pltpu.VMEM((2, 8, 8, 128), jnp.float32),
            pltpu.VMEM((2 + NP, 24, 8, 128), jnp.int32),
            pltpu.VMEM((2 + NP, 8, 128), jnp.float32),
            pltpu.SemaphoreType.DMA((2, NP, 2)),
            pltpu.SemaphoreType.DMA((5, 2)),
        ],
        compiler_params=pltpu.CompilerParams(vmem_limit_bytes=127 * 1024 * 1024),
    )(A_x, _tiles_k(A_k_cache), _tiles_k(A_v_cache), _tiles_w(A_wq), _tiles_w(A_wo),
      _tiles_w(B_w3), _tiles_w(B_w4))
```

```python
import contextlib, math
import jax
import jax.numpy as jnp
import numpy as np
from jax import lax
from jax.experimental import pallas as pl
from jax.experimental.pallas import tpu as pltpu

D = 640; NH = 32; DH = 192; SK = 32768; W = 4096; FF = 1536
NP = NH // 2; NCB = W // 128; CB0 = (SK - W) // 128
ND = D // 128
EPS = 1e-5
LOG2E = 1.4426950408889634
QSCALE = (DH ** -0.5) * LOG2E
_MASK_HI = np.int32(-65536)
NT = (((1,), (1,)), ((), ()))

DEFAULT = dict(AG=6, scopes=False, flags=None,
               push=0.85, lat=150, rev_until=150, stepc=9.0, t0=15, order="q,z,k0,w,k1", fwd=True, rev=True,
               xpose=2.0, tie_every=1, fuse=True, rev_per=1)


def _tiles_k(c):
    t = jnp.transpose(c[0], (0, 2, 1)).reshape(NP, 24, 2, 8, SK // 128, 128)
    return jnp.transpose(t, (0, 1, 2, 4, 3, 5))


def _tiles_w(w):
    k, n = w.shape
    return jnp.transpose(w.reshape(k // 16, 2, 8, n // 128, 128), (0, 1, 3, 2, 4))


def _as_bf16(words):
    n = words.shape[0]
    return pltpu.bitcast(words.reshape(n * 8, 128), jnp.bfloat16)


def _mm(a, b):
    return jnp.dot(a, b, preferred_element_type=jnp.float32)


def _layernorm(x):
    m = jnp.mean(x, axis=-1, keepdims=True)
    d = x - m
    v = jnp.mean(d * d, axis=-1, keepdims=True)
    return d * lax.rsqrt(v + EPS)


def _gelu(x):
    c = np.float32(0.7978845608028654)
    return 0.5 * x * (1.0 + jnp.tanh(c * (x + np.float32(0.044715) * (x * x * x))))


def _pack16(row8):
    raise NotImplementedError


def make_kernel(cfg):
    AG = cfg["AG"]
    scope = jax.named_scope if cfg["scopes"] else (lambda n: contextlib.nullcontext())

    def _kernel(x_hbm, k_hbm, v_hbm, wq_hbm, wo_hbm, w3_hbm, w4_hbm, o_ref,
                xbuf, kbuf, vbuf, wqbuf, wobuf, w3buf, w4buf, lbuf, pbuf, zbuf, ibuf, mlbuf, obuf, ybuf, sbuf, xbuf2,
                kv_sem, w_sem):
        ki = k_hbm.bitcast(jnp.int32)
        vi = v_hbm.bitcast(jnp.int32)

        def kv_copy(t, g, b):
            src, dst = ((ki, kbuf), (vi, vbuf))[t]
            return pltpu.make_async_copy(src.at[g, :, b, pl.ds(CB0, NCB)],
                                         dst.at[g, :, :, pl.ds(4 * b, 4), :], kv_sem.at[t, g, b])

        def w_copy(i, b):
            src, dst = ((wq_hbm, wqbuf), (wo_hbm, wobuf), (w3_hbm, w3buf), (w4_hbm, w4buf))[i]
            return pltpu.make_async_copy(src.bitcast(jnp.int32).at[:, b],
                                         dst.at[:, :, pl.ds(4 * b, 4), :], w_sem.at[i, b])

        x_copy = pltpu.make_async_copy(x_hbm, xbuf, w_sem.at[4, 0])
        x_copy.start()
        for b in range(2):
            w_copy(0, b).start()
        for g in range(NP):
            for t in range(2):
                for b in range(2):
                    kv_copy(t, g, b).start()
        for i in (1, 2, 3):
            for b in range(2):
                w_copy(i, b).start()

        def wait_w(i):
            for b in range(2):
                w_copy(i, b).wait()

        def wait_kv(t, g):
            for b in range(2):
                kv_copy(t, g, b).wait()

        rows = lax.broadcasted_iota(jnp.int32, (8, 128), 0)
        lanes = lax.broadcasted_iota(jnp.int32, (8, 128), 1)
        lane_lo = lanes < 64

        def pack2(lo, hi):
            return pltpu.bitcast(pltpu.pack_elementwise([lo, hi], packed_dtype=jnp.bfloat16), jnp.int32)

        def to_words(v8):
            return pack2(v8, v8)

        def lhs_of(words):
            return jnp.concatenate([pltpu.bitcast(w, jnp.bfloat16) for w in words], axis=1)

        def mm8(words, rhs):
            return _mm(lhs_of(words), rhs)[0:8]

        def store_L(g, q):
            z = jnp.zeros((8, 128), jnp.float32)
            w = [pack2(q[0], z), pack2(jnp.where(lane_lo, q[1], 0.0), jnp.where(lane_lo, 0.0, q[1])), pack2(z, q[2])]
            for r in range(4):
                for t in range(3):
                    lbuf[g, r, t] = jnp.where(rows == r, w[t], 0)

        def store_y(y):
            for k in range(ND):
                ybuf[k] = to_words(y[:, 128 * k:128 * k + 128])

        def q_tile(g, c, tie=None):
            yw = [ybuf[k] for k in range(ND)]
            if tie is not None:
                yw = [tie(w) for w in yw]
            return mm8(yw, _as_bf16(wqbuf[:, 3 * g + c])) * np.float32(QSCALE)

        def make_q(g):
            store_L(g, [q_tile(g, c) for c in range(3)])

        def qk_block(g, cb, tie=None):
            lw = [lbuf[g, cb % 4, t] for t in range(3)]
            if tie is not None:
                lw = [tie(w) for w in lw]
            return mm8(lw, _as_bf16(kbuf[g, :, cb]))

        def qk_all(g):
            out = []
            for i in range(8):
                tot = None
                for r in range(4):
                    s = qk_block(g, 4 * i + r)
                    tot = s if tot is None else tot + s
                out.append(tot)
            return out

        def softmax_to(slot, g, sc, m=None):
            if sc is None:
                sc = [sbuf[i] for i in range(8)]
            else:
                m = sc[0]
                for s in sc[1:]:
                    m = jnp.maximum(m, s)
            m = jnp.maximum(m, pltpu.roll(m, 2, 0))
            m = jnp.maximum(m, pltpu.roll(m, 4, 0))
            tot = None
            for i in range(8):
                p = jnp.exp2(sc[i] - m)
                pbuf[slot, 8 * i:8 * i + 8, :] = p
                tot = p if tot is None else tot + p
            tot = tot + pltpu.roll(tot, 2, 0)
            tot = tot + pltpu.roll(tot, 4, 0)
            mlbuf[g, 0] = m
            mlbuf[g, 1] = tot

        def lane_weights(g, slot):
            m = mlbuf[g, 0]
            M = jnp.max(m, axis=1, keepdims=True)
            c = jnp.exp2(m - M)
            L = jnp.sum(c * mlbuf[g, 1], axis=1, keepdims=True)
            ibuf[slot, 0:8, :] = c / L

        def pv_steps(g, slot, zslot):
            hook = None
            for e in range(2):
                for a0 in range(0, 12, AG):
                    acc = [[None, None] for _ in range(AG)]
                    for cb in range(NCB):
                        row = 8 * (cb // 4) + 2 * (cb % 4) + e
                        p = pbuf[slot, pl.ds(row, 8, stride=0), :]
                        hook = yield (acc, )
                        if hook is not None:
                            p = hook(p)
                        for a in range(AG):
                            w = vbuf[g, 12 * e + a0 + a, cb]
                            lo = pltpu.bitcast(w << 16, jnp.float32) * p
                            hi = pltpu.bitcast(w & _MASK_HI, jnp.float32) * p
                            A = acc[a]
                            A[0] = lo if A[0] is None else A[0] + lo
                            A[1] = hi if A[1] is None else A[1] + hi
                    for a in range(AG):
                        z = pltpu.pack_elementwise(acc[a], packed_dtype=jnp.bfloat16)
                        zbuf[zslot, 12 * e + a0 + a] = pltpu.bitcast(z, jnp.int32)
            yield None

        def pv_all(g, slot, zslot):
            gen = pv_steps(g, slot, zslot)
            st = next(gen)
            while st is not None:
                st = gen.send(None)

        def o_rows(zslot, tie=None):
            wa = ibuf[zslot, pl.ds(0, 8, stride=0), :]
            wb = ibuf[zslot, pl.ds(1, 8, stride=0), :]
            pa, pb = pack2(wa, wa), pack2(wb, wb)
            lw = [pa, jnp.where(rows < 2, pa, pb), pb]
            if tie is not None:
                lw = [tie(w) for w in lw]
            o = []
            for t in range(3):
                z = _as_bf16(zbuf[zslot, 8 * t:8 * t + 8])
                o.append(lax.dot_general(pltpu.bitcast(lw[t], jnp.bfloat16), z, NT,
                                         preferred_element_type=jnp.float32)[0:8])
            o[1] = jnp.where((rows < 4) == lane_lo, o[1], pltpu.roll(o[1], 4, 0))
            return o

        def store_o(slot, o):
            for t in range(3):
                obuf[slot, t] = to_words(o[t])

        def wo_tile(slot, g, c):
            return mm8([obuf[slot, t] for t in range(3)], _as_bf16(wobuf[pl.ds(24 * g, 24), c]))

        x_copy.wait()
        x = jnp.broadcast_to(xbuf[0].astype(jnp.float32), (8, D))
        pbuf[:, 64:72, :] = jnp.zeros((2, 8, 128), jnp.float32)
        ibuf[0] = jnp.zeros((16, 128), jnp.float32)
        ibuf[:, 8:16, :] = jnp.zeros((NP + 1, 8, 128), jnp.float32)
        zbuf[0] = jnp.zeros((24, 8, 128), jnp.int32)
        zero = jnp.zeros((8, 128), jnp.float32)

        def attn_first(x):
            store_y(_layernorm(x))
            wait_w(0)

            def q_body(g, c):
                make_q(g)
                return c
            with scope("q1"):
                lax.fori_loop(0, NP, q_body, 0)
            with scope("qk0_1"):
                wait_kv(0, 0)
                softmax_to(0, 0, qk_all(0))

            def body(g, c):
                slot = g & 1
                gn = jnp.minimum(g + 1, NP - 1)

                @pl.when(g + 1 < NP)
                def _():
                    wait_kv(0, g + 1)
                wait_kv(1, g)
                sc = qk_all(gn)
                lane_weights(g, g + 1)
                pv_all(g, slot, g + 1)
                softmax_to(1 - slot, gn, sc)
                return c
            with scope("main1"):
                lax.fori_loop(0, NP, body, 0)

            def orow_body(g, c):
                store_o(g, o_rows(g + 1))
                return c
            with scope("orows1"):
                lax.fori_loop(0, NP, orow_body, 0)
            with scope("waitwo1"):
                wait_w(1)

            def wo_body(i, xacc):
                xacc = list(xacc)
                for j in range(4):
                    g = i * 4 + j
                    for c in range(ND):
                        xacc[c] = xacc[c] + wo_tile(g, g, c)
                return tuple(xacc)
            with scope("oproj1"):
                xacc = lax.fori_loop(0, NP // 4, wo_body, (zero,) * ND)
            return x + jnp.concatenate(xacc, axis=1)

        def attn_second(x):
            store_y(_layernorm(x))
            with scope("q2"):
                make_q(0)
                make_q(1)
            with scope("qk0_2"):
                softmax_to(0, 0, qk_all(0))
            for c in range(ND):
                xbuf2[c] = zero

            def body(g, carry):
                slot = g & 1
                gn = jnp.minimum(g + 1, NP - 1)
                gq = jnp.minimum(g + 2, NP - 1)
                gp = jnp.maximum(g - 1, 0)
                msk = pbuf[0, 64:72, :] == 0.0
                lane_weights(g, g + 1)
                st = {"sc": [None] * 8, "q": [None] * 3, "m": None}

                def mk_tie(av):
                    if av is None:
                        return None
                    per = cfg["rev_per"]

                    def tie(w):
                        for _ in range(per):
                            flat = av[0]
                            w = jnp.where(msk, w, pltpu.bitcast(flat[av[1][0] % len(flat)], jnp.int32))
                            av[1][0] += 1
                        return w
                    return tie

                tasks = []

                def t_q(c):
                    def fn(av):
                        r = q_tile(gq, c, mk_tie(av))
                        st["q"][c] = r
                        if c == 2:
                            store_L(gq, st["q"])
                        return r
                    return (40, fn)

                def t_z():
                    def fn(av):
                        o = o_rows(g, mk_tie(av))
                        store_o(0, o)
                        return o[2]
                    return (24 * cfg["xpose"], fn)

                def t_w(c):
                    def fn(av):
                        r = xbuf2[c] + wo_tile(0, gp, c)
                        xbuf2[c] = r
                        return r
                    return (24, fn)

                def t_k(cb):
                    def fn(av):
                        i, r = divmod(cb, 4)
                        s = qk_block(gn, cb, mk_tie(av))
                        st["sc"][i] = s if r == 0 else st["sc"][i] + s
                        if r == 3:
                            sbuf[i] = st["sc"][i]
                            st["m"] = st["sc"][i] if st["m"] is None else jnp.maximum(st["m"], st["sc"][i])
                            return st["m"]
                        return st["sc"][i]
                    return (24, fn)

                for name in cfg["order"].split(","):
                    if name == "q": tasks += [t_q(c) for c in range(3)]
                    elif name == "z": tasks += [t_z()]
                    elif name == "w": tasks += [t_w(c) for c in range(ND)]
                    elif name == "k0": tasks += [t_k(cb) for cb in range(16)]
                    elif name == "k1": tasks += [t_k(cb) for cb in range(16, 32)]
                    elif name == "k": tasks += [t_k(cb) for cb in range(32)]

                issue = []
                t = cfg["t0"]
                for n, fn in tasks:
                    t += n * cfg["push"]
                    issue.append(t)
                gen = pv_steps(g, slot, g + 1)
                state = next(gen)
                step = 0
                nxt = 0
                pending = []
                last_acc = None
                rot = [0]
                nsteps = 64 * (12 // AG)
                cnt = 0
                while state is not None:
                    now = cfg["t0"] + cfg["stepc"] * step
                    acc = state[0]
                    if acc[0][0] is not None:
                        last_acc = ([v for pair in acc for v in pair], rot)
                    while nxt < len(tasks) and (issue[nxt] <= now + cfg["stepc"] or step == nsteps - 1):
                        av = last_acc if (cfg["rev"] and issue[nxt] <= cfg["rev_until"]) else None
                        val = tasks[nxt][1](av)
                        cnt += 1
                        if val is not None and (cnt % cfg["tie_every"] == 0):
                            pending.append((issue[nxt] + cfg["lat"], val))
                        nxt += 1
                    ready = [v for (tt, v) in pending if tt <= now or step == nsteps - 1]
                    pending = [(tt, v) for (tt, v) in pending if not (tt <= now or step == nsteps - 1)]

                    def hook(p, ready=ready):
                        if cfg["fwd"]:
                            for v in ready:
                                p = jnp.where(msk, p, v)
                        return p
                    state = gen.send(hook)
                    step += 1
                assert nxt == len(tasks)
                softmax_to(1 - slot, gn, None, st["m"])
                return carry

            with scope("main2"):
                lax.fori_loop(0, NP, body, 0)
            with scope("oproj2"):
                store_o(0, o_rows(NP))
                xacc = [xbuf2[c] + wo_tile(0, NP - 1, c) for c in range(ND)]
            return x + jnp.concatenate(xacc, axis=1)

        def mlp_layer(x, first):
            y = _layernorm(x)
            u_bf = _layernorm(y).astype(jnp.bfloat16)
            if first:
                wait_w(2)
            h = jnp.concatenate([_mm(u_bf, _as_bf16(w3buf[:, c])) for c in range(FF // 128)], axis=1)
            h_bf = _gelu(h).astype(jnp.bfloat16)
            if first:
                wait_w(3)
            h2 = jnp.concatenate([_mm(h_bf, _as_bf16(w4buf[:, c])) for c in range(D // 128)], axis=1)
            return x + (y + h2)

        x = attn_first(x)
        with scope("mlp1"):
            x = mlp_layer(x, True)
        x = attn_second(x)
        with scope("mlp2"):
            x = mlp_layer(x, False)
        o_ref[0] = x[0:1, :].astype(o_ref.dtype)
    return _kernel


_CFG = dict(DEFAULT)
_CFG.update(dict(order='z,k0,w,k1,q',push=1.0,stepc=9.3,lat=150,rev_until=200,rev_per=2))
_KERNEL = make_kernel(_CFG)

@jax.jit
def pallas_interleave_layers__sliding_block_cached__mixer_s_mlp__decode_kernel(A_x, A_k_cache, A_v_cache, A_wq, A_wo, B_x, B_w1, B_w2, B_w3, B_w4):
    any_spec = pl.BlockSpec(memory_space=pl.ANY)
    return pl.pallas_call(
        _KERNEL,
        out_shape=jax.ShapeDtypeStruct((1, 1, D), A_x.dtype),
        in_specs=[any_spec] * 7,
        out_specs=pl.BlockSpec(memory_space=pltpu.VMEM),
        scratch_shapes=[
            pltpu.VMEM((1, 1, D), jnp.bfloat16),
            pltpu.VMEM((NP, 24, NCB, 8, 128), jnp.int32),
            pltpu.VMEM((NP, 24, NCB, 8, 128), jnp.int32),
            pltpu.VMEM((D // 16, NH * DH // 128, 8, 128), jnp.int32),
            pltpu.VMEM((NH * DH // 16, D // 128, 8, 128), jnp.int32),
            pltpu.VMEM((D // 16, FF // 128, 8, 128), jnp.int32),
            pltpu.VMEM((FF // 16, D // 128, 8, 128), jnp.int32),
            pltpu.VMEM((NP, 4, 3, 8, 128), jnp.int32),
            pltpu.VMEM((2, 72, 128), jnp.float32),
            pltpu.VMEM((NP + 1, 24, 8, 128), jnp.int32),
            pltpu.VMEM((NP + 1, 16, 128), jnp.float32),
            pltpu.VMEM((NP, 2, 8, 128), jnp.float32),
            pltpu.VMEM((NP, 3, 8, 128), jnp.int32),
            pltpu.VMEM((ND, 8, 128), jnp.int32),
            pltpu.VMEM((8, 8, 128), jnp.float32),
            pltpu.VMEM((ND, 8, 128), jnp.float32),
            pltpu.SemaphoreType.DMA((2, NP, 2)),
            pltpu.SemaphoreType.DMA((5, 2)),
        ],
        compiler_params=pltpu.CompilerParams(vmem_limit_bytes=127 * 1024 * 1024, flags=_CFG["flags"]),
    )(A_x, _tiles_k(A_k_cache), _tiles_k(A_v_cache), _tiles_w(A_wq), _tiles_w(A_wo),
      _tiles_w(B_w3), _tiles_w(B_w4))
```

```python
import functools

import jax
import jax.numpy as jnp
import numpy as np
from jax import lax
from jax.experimental import pallas as pl
from jax.experimental.pallas import tpu as pltpu

D = 640
NH = 32
DH = 192
SK = 32768
W = 4096
FF = 1536
NP = NH // 2
NCB = W // 128
CB0 = (SK - W) // 128
ND = D // 128
NF = FF // 128
EPS = 1e-5
QSCALE = np.float32((DH ** -0.5) * 1.4426950408889634)
NT = (((1,), (1,)), ((), ()))

V_CHUNKS = (0, 8, 16)
W4_CHUNKS = (0, 48, 80, 96)
NV = len(V_CHUNKS) - 1
NW4 = len(W4_CHUNKS) - 1

AG = 4
T0 = 15
STEP = 6.2
PUSH = 1.0
XPOSE = 2.0
LAT = 170
REV_UNTIL = 240
REV_PER = 2
ORDER_LAYER1 = ("z", "k")
ORDER_LAYER2 = ("z", "k0", "w", "k1", "q")


def _tiles_cache(c):
    t = jnp.transpose(c[0], (0, 2, 1)).reshape(NP, 24, 2, 8, SK // 128, 128)
    return jnp.transpose(t, (0, 1, 2, 4, 3, 5))


def _tiles_weight(w):
    k, n = w.shape
    return jnp.transpose(w.reshape(k // 16, 2, 8, n // 128, 128), (0, 1, 3, 2, 4))


def _as_bf16(words):
    n = words.shape[0]
    return pltpu.bitcast(words.reshape(n * 8, 128), jnp.bfloat16)


def _mm(a, b):
    return jnp.dot(a, b, preferred_element_type=jnp.float32)


def _layernorm(x):
    m = jnp.mean(x, axis=-1, keepdims=True)
    d = x - m
    v = jnp.mean(d * d, axis=-1, keepdims=True)
    return d * lax.rsqrt(v + EPS)


def _ln_stats(x):
    m = jnp.mean(x, axis=-1, keepdims=True)
    d = x - m
    s1 = jnp.mean(d, axis=-1, keepdims=True)
    s2 = jnp.mean(d * d, axis=-1, keepdims=True)
    r = lax.rsqrt(s2 + EPS)
    r2 = lax.rsqrt(r * r * (s2 - s1 * s1) + EPS)
    return m, s1, r, r2


def _gelu(x):
    c = np.float32(0.7978845608028654)
    return 0.5 * x * (1.0 + jnp.tanh(c * (x + np.float32(0.044715) * (x * x * x))))


def _lhs_tiles(x):
    return [x[:, 128 * k:128 * k + 128].astype(jnp.bfloat16) for k in range(ND)]


def _kernel(x_hbm, k_hbm, v_hbm, wq_hbm, wo_hbm, w3_hbm, w4_hbm, o_ref,
            xbuf, kbuf, vbuf, wqbuf, wobuf, w3buf, w4buf,
            lbuf, pbuf, zbuf, ibuf, mlbuf, obuf, ybuf, sbuf, xacc_buf, csbuf, sems):
    ki = k_hbm.bitcast(jnp.int32)
    vi = v_hbm.bitcast(jnp.int32)

    def kv_copy(t, i, b):
        src, dst, ch = ((ki, kbuf, (0, NP)), (vi, vbuf, V_CHUNKS))[t]
        g0, n = ch[i], ch[i + 1] - ch[i]
        return pltpu.make_async_copy(src.at[pl.ds(g0, n), :, b, pl.ds(CB0, NCB)],
                                     dst.at[pl.ds(g0, n), :, :, pl.ds(4 * b, 4), :],
                                     sems.at[0 if t == 0 else i])

    def w_copy(i, b, part=None):
        src, dst = ((wq_hbm, wqbuf), (wo_hbm, wobuf), (w3_hbm, w3buf), (w4_hbm, w4buf))[i]
        src = src.bitcast(jnp.int32)
        if part is None:
            return pltpu.make_async_copy(src.at[:, b], dst.at[:, :, pl.ds(4 * b, 4), :],
                                         sems.at[0 if i == 0 else NV + i - 1])
        a0, n = W4_CHUNKS[part], W4_CHUNKS[part + 1] - W4_CHUNKS[part]
        return pltpu.make_async_copy(src.at[pl.ds(a0, n), b],
                                     dst.at[pl.ds(a0, n), :, pl.ds(4 * b, 4), :],
                                     sems.at[NV + 2 + part])

    x_copy = pltpu.make_async_copy(x_hbm, xbuf, sems.at[0])
    x_copy.start()
    for b in range(2):
        w_copy(0, b).start()
    for t, i in [(0, 0)] + [(1, i) for i in range(NV)]:
        for b in range(2):
            kv_copy(t, i, b).start()
    for i in (1, 2):
        for b in range(2):
            w_copy(i, b).start()
    for part in range(NW4):
        for b in range(2):
            w_copy(3, b, part).start()

    def wait_w(i, part=None):
        for b in range(2):
            w_copy(i, b, part).wait()

    def wait_kv(t, i):
        for b in range(2):
            kv_copy(t, i, b).wait()

    rows = lax.broadcasted_iota(jnp.int32, (8, 128), 0)
    lanes = lax.broadcasted_iota(jnp.int32, (8, 128), 1)
    lane_lo = lanes < 64

    def mm_tiles(lhs, rhs_words, tie=None):
        tot = None
        for t, l in enumerate(lhs):
            w = [rhs_words[8 * t + i] for i in range(8)]
            if tie is not None:
                w[0] = tie(w[0])
            r = _mm(l, pltpu.bitcast(jnp.concatenate(w, axis=0), jnp.bfloat16))
            tot = r if tot is None else tot + r
        return tot

    def store_L(g, q):
        for r in range(4):
            ra = rows == 2 * r
            rb = rows == 2 * r + 1
            lbuf[g, r, 0] = jnp.where(ra, q[0], 0.0).astype(jnp.bfloat16)
            lbuf[g, r, 1] = jnp.where((ra & lane_lo) | (rb & (~lane_lo)), q[1], 0.0).astype(jnp.bfloat16)
            lbuf[g, r, 2] = jnp.where(rb, q[2], 0.0).astype(jnp.bfloat16)

    def store_y(y):
        for k, t in enumerate(_lhs_tiles(y)):
            ybuf[k] = t

    def q_tile(g, c, tie=None):
        return mm_tiles([ybuf[k] for k in range(ND)], wqbuf[:, 3 * g + c], tie) * QSCALE

    def make_q(g):
        store_L(g, [q_tile(g, c) for c in range(3)])

    def qk_block(g, cb, tie=None):
        return mm_tiles([lbuf[g, cb % 4, t] for t in range(3)], kbuf[g, :, cb], tie)

    def qk_all(g):
        out = []
        for i in range(8):
            tot = None
            for r in range(4):
                s = qk_block(g, 4 * i + r)
                tot = s if tot is None else tot + s
            out.append(tot)
        return out

    def softmax_to(slot, g, sc, m=None):
        if sc is None:
            sc = [sbuf[i] for i in range(8)]
        else:
            m = sc[0]
            for s in sc[1:]:
                m = jnp.maximum(m, s)
        m = jnp.maximum(m, pltpu.roll(m, 2, 0))
        m = jnp.maximum(m, pltpu.roll(m, 4, 0))
        tot = None
        for i in range(8):
            p = jnp.exp2(sc[i] - m)
            pbuf[slot, 8 * i:8 * i + 8, :] = p
            tot = p if tot is None else tot + p
        tot = tot + pltpu.roll(tot, 2, 0)
        tot = tot + pltpu.roll(tot, 4, 0)
        mlbuf[g, 0] = m
        mlbuf[g, 1] = tot

    def lane_weights(g, slot):
        m = mlbuf[g, 0]
        M = jnp.max(m, axis=1, keepdims=True)
        c = jnp.exp2(m - M)
        L = jnp.sum(c * mlbuf[g, 1], axis=1, keepdims=True)
        ibuf[slot, 0:8, :] = c / L

    def pv_steps(g, slot, zslot):
        for e in range(2):
            for a0 in range(0, 12, AG):
                acc = [None] * AG
                for cb in range(NCB):
                    row = 8 * (cb // 4) + 2 * (cb % 4) + e
                    p = pbuf[slot, pl.ds(row, 8, stride=0), :]
                    hook = yield acc
                    p = hook(p)
                    p = jnp.concatenate([p, p], axis=0)
                    for a in range(AG):
                        w = vbuf[g, 12 * e + a0 + a, cb]
                        t = pltpu.bitcast(w, jnp.bfloat16).astype(jnp.float32) * p
                        acc[a] = t if acc[a] is None else acc[a] + t
                for a in range(AG):
                    zbuf[zslot, pl.ds(16 * (12 * e + a0 + a), 16), :] = acc[a]
        yield None

    def o_rows(zslot, tie=None):
        wa = ibuf[zslot, pl.ds(0, 8, stride=0), :]
        wb = ibuf[zslot, pl.ds(1, 8, stride=0), :]
        lw = [wa.astype(jnp.bfloat16), jnp.where(rows < 4, wa, wb).astype(jnp.bfloat16),
              wb.astype(jnp.bfloat16)]
        o = []
        for t in range(3):
            z = zbuf[zslot, pl.ds(128 * t, 128), :]
            if tie is not None:
                z0 = pltpu.bitcast(tie(pltpu.bitcast(z[0:8], jnp.int32)), jnp.float32)
                z = jnp.concatenate([z0, z[8:]], axis=0)
            z = z.astype(jnp.bfloat16)
            o.append(lax.dot_general(lw[t], z, NT, preferred_element_type=jnp.float32))
        o[1] = jnp.where((rows < 4) == lane_lo, o[1], pltpu.roll(o[1], 4, 0))
        return o

    def store_o(slot, o):
        for t in range(3):
            obuf[slot, t] = o[t].astype(jnp.bfloat16)

    def wo_tile(slot, g, c):
        return mm_tiles([obuf[slot, t] for t in range(3)], wobuf[pl.ds(24 * g, 24), c])

    x_copy.wait()
    wait_w(0)
    wait_kv(0, 0)
    wait_kv(1, 0)
    x = jnp.broadcast_to(xbuf[0].astype(jnp.float32), (8, D))
    pbuf[:, 64:72, :] = jnp.zeros((2, 8, 128), jnp.float32)
    ibuf[0] = jnp.zeros((16, 128), jnp.float32)
    ibuf[:, 8:16, :] = jnp.zeros((NP + 1, 8, 128), jnp.float32)
    zbuf[0] = jnp.zeros((384, 128), jnp.float32)
    zero = jnp.zeros((8, 128), jnp.float32)

    def body(g, order):
        slot = g & 1
        gn = jnp.minimum(g + 1, NP - 1)
        gq = jnp.minimum(g + 2, NP - 1)
        gp = jnp.maximum(g - 1, 0)
        true = pbuf[0, 64:72, :] == 0.0
        lane_weights(g, g + 1)
        st = {"sc": [None] * 8, "q": [None] * 3, "m": None}

        def mk_tie(av):
            if av is None:
                return None

            def tie(w):
                for _ in range(REV_PER):
                    flat, rot = av
                    w = jnp.where(true, w, pltpu.bitcast(flat[rot[0] % len(flat)], jnp.int32))
                    rot[0] += 1
                return w
            return tie

        def t_q(c):
            def fn(av):
                r = q_tile(gq, c, mk_tie(av))
                st["q"][c] = r
                if c == 2:
                    store_L(gq, st["q"])
                return r
            return (40, fn)

        def t_z():
            def fn(av):
                o = o_rows(g, mk_tie(av))
                store_o(g, o)
                return o[2]
            return (24 * XPOSE, fn)

        def t_w(c):
            def fn(av):
                r = xacc_buf[c] + wo_tile(g, gp, c)
                xacc_buf[c] = r
                return r
            return (24, fn)

        def t_k(cb):
            def fn(av):
                i, r = divmod(cb, 4)
                s = qk_block(gn, cb, mk_tie(av))
                st["sc"][i] = s if r == 0 else st["sc"][i] + s
                if r == 3:
                    sbuf[i] = st["sc"][i]
                    st["m"] = st["sc"][i] if st["m"] is None else jnp.maximum(st["m"], st["sc"][i])
                    return st["m"]
                return st["sc"][i]
            return (24, fn)

        groups = {"q": lambda: [t_q(c) for c in range(3)], "z": lambda: [t_z()],
                  "w": lambda: [t_w(c) for c in range(ND)],
                  "k0": lambda: [t_k(cb) for cb in range(16)],
                  "k1": lambda: [t_k(cb) for cb in range(16, 32)],
                  "k": lambda: [t_k(cb) for cb in range(32)]}
        tasks = [t for name in order for t in groups[name]()]
        issue, t = [], T0
        for n, _ in tasks:
            t += n * PUSH
            issue.append(t)

        gen = pv_steps(g, slot, g + 1)
        acc = next(gen)
        nsteps = 64 * (12 // AG)
        step, nxt, pending, last_acc, rot = 0, 0, [], None, [0]
        while acc is not None:
            now = T0 + STEP * step
            last = step == nsteps - 1
            if acc[0] is not None:
                last_acc = ([h for v in acc for h in (v[0:8], v[8:16])], rot)
            while nxt < len(tasks) and (issue[nxt] <= now + STEP or last):
                val = tasks[nxt][1](last_acc if issue[nxt] <= REV_UNTIL else None)
                pending.append((issue[nxt] + LAT, val))
                nxt += 1
            ready = [v for tt, v in pending if tt <= now or last]
            pending = [(tt, v) for tt, v in pending if not (tt <= now or last)]

            def hook(p, ready=ready):
                for v in ready:
                    p = jnp.where(true, p, v)
                return p
            acc = gen.send(hook)
            step += 1
        softmax_to(1 - slot, gn, None, st["m"])

    def attn_first(x):
        store_y(_layernorm(x))
        ones = [jnp.ones((8, 128), jnp.bfloat16)] * ND
        for c in range(3):
            csbuf[c] = mm_tiles(ones, wqbuf[:, c])

        def q_body(g, c):
            make_q(g)
            return c
        lax.fori_loop(0, NP, q_body, 0)
        softmax_to(0, 0, qk_all(0))

        def loop(g, c):
            for i in range(1, NV):
                pl.when(g == V_CHUNKS[i])(functools.partial(wait_kv, 1, i))
            body(g, ORDER_LAYER1)
            return c
        lax.fori_loop(0, NP, loop, 0)
        store_o(NP, o_rows(NP))
        wait_w(1)

        def wo_body(i, xacc):
            xacc = list(xacc)
            for j in range(4):
                g = i * 4 + j
                for c in range(ND):
                    xacc[c] = xacc[c] + wo_tile(g + 1, g, c)
            return tuple(xacc)
        xacc = lax.fori_loop(0, NP // 4, wo_body, (zero,) * ND)
        return x + jnp.concatenate(xacc, axis=1)

    def attn_second(x):
        xb = _lhs_tiles(x)
        raw = [mm_tiles(xb, wqbuf[:, c]) for c in range(3)]
        m, _, r, _ = _ln_stats(x)
        store_L(0, [(raw[c] - m * csbuf[c]) * (r * QSCALE) for c in range(3)])
        store_y((x - m) * r)
        make_q(1)
        softmax_to(0, 0, qk_all(0))
        for c in range(ND):
            xacc_buf[c] = zero

        def loop(g, c):
            body(g, ORDER_LAYER2)
            return c
        lax.fori_loop(0, NP, loop, 0)
        store_o(NP, o_rows(NP))
        xacc = [xacc_buf[c] + wo_tile(NP, NP - 1, c) for c in range(ND)]
        return x + jnp.concatenate(xacc, axis=1)

    def mlp_layer(x, first):
        m, s1, r, r2 = _ln_stats(x)
        y = (x - m) * r
        if first:
            wait_w(2)
            ub = _lhs_tiles((x - m - s1) * (r * r2))
            h = jnp.concatenate([mm_tiles(ub, w3buf[:, c]) for c in range(NF)], axis=1)
        else:
            xb = _lhs_tiles(x)
            raw = [mm_tiles(xb, w3buf[:, c]) for c in range(NF)]
            h = jnp.concatenate([(raw[c] - (m + s1) * csbuf[3 + c]) * (r * r2) for c in range(NF)],
                                axis=1)
        h_bf = _gelu(h).astype(jnp.bfloat16)
        if first:
            ones = [jnp.ones((8, 128), jnp.bfloat16)] * ND
            for c in range(NF):
                csbuf[3 + c] = mm_tiles(ones, w3buf[:, c])
        h2 = [None] * ND
        chunks = W4_CHUNKS if first else (0, FF // 16)
        for part in range(len(chunks) - 1):
            if first:
                wait_w(3, part)
            a0, a1 = chunks[part], chunks[part + 1]
            for c in range(ND):
                t = _mm(h_bf[:, 16 * a0:16 * a1], _as_bf16(w4buf[a0:a1, c]))
                h2[c] = t if h2[c] is None else h2[c] + t
        return x + (y + jnp.concatenate(h2, axis=1))

    x = attn_first(x)
    x = mlp_layer(x, True)
    x = attn_second(x)
    x = mlp_layer(x, False)
    o_ref[0] = x[0:1, :].astype(o_ref.dtype)


@jax.jit
def pallas_interleave_layers__sliding_block_cached__mixer_s_mlp__decode_kernel(
    A_x: jax.Array,
    A_k_cache: jax.Array,
    A_v_cache: jax.Array,
    A_wq: jax.Array,
    A_wo: jax.Array,
    B_x: jax.Array,
    B_w1: jax.Array,
    B_w2: jax.Array,
    B_w3: jax.Array,
    B_w4: jax.Array,
):
    del B_x, B_w1, B_w2
    return pl.pallas_call(
        _kernel,
        out_shape=jax.ShapeDtypeStruct((1, 1, D), A_x.dtype),
        in_specs=[pl.BlockSpec(memory_space=pl.ANY)] * 7,
        out_specs=pl.BlockSpec(memory_space=pltpu.VMEM),
        scratch_shapes=[
            pltpu.VMEM((1, 1, D), jnp.bfloat16),
            pltpu.VMEM((NP, 24, NCB, 8, 128), jnp.int32),
            pltpu.VMEM((NP, 24, NCB, 8, 128), jnp.int32),
            pltpu.VMEM((D // 16, NH * DH // 128, 8, 128), jnp.int32),
            pltpu.VMEM((NH * DH // 16, ND, 8, 128), jnp.int32),
            pltpu.VMEM((D // 16, NF, 8, 128), jnp.int32),
            pltpu.VMEM((FF // 16, ND, 8, 128), jnp.int32),
            pltpu.VMEM((NP, 4, 3, 8, 128), jnp.bfloat16),
            pltpu.VMEM((2, 72, 128), jnp.float32),
            pltpu.VMEM((NP + 1, 384, 128), jnp.float32),
            pltpu.VMEM((NP + 1, 16, 128), jnp.float32),
            pltpu.VMEM((NP, 2, 8, 128), jnp.float32),
            pltpu.VMEM((NP + 1, 3, 8, 128), jnp.bfloat16),
            pltpu.VMEM((ND, 8, 128), jnp.bfloat16),
            pltpu.VMEM((8, 8, 128), jnp.float32),
            pltpu.VMEM((ND, 8, 128), jnp.float32),
            pltpu.VMEM((3 + NF, 8, 128), jnp.float32),
            pltpu.SemaphoreType.DMA((NV + 2 + NW4,)),
        ],
        compiler_params=pltpu.CompilerParams(vmem_limit_bytes=127 * 1024 * 1024),
    )(A_x, _tiles_cache(A_k_cache), _tiles_cache(A_v_cache), _tiles_weight(A_wq),
      _tiles_weight(A_wo), _tiles_weight(B_w3), _tiles_weight(B_w4))
```

```python
import functools

import jax
import jax.numpy as jnp
import numpy as np
from jax import lax
from jax.experimental import pallas as pl
from jax.experimental.pallas import tpu as pltpu

D = 640
NH = 32
DH = 192
SK = 32768
W = 4096
FF = 1536
NP = NH // 2
NCB = W // 128
CB0 = (SK - W) // 128
ND = D // 128
NF = FF // 128
EPS = 1e-5
QSCALE = np.float32((DH ** -0.5) * 1.4426950408889634)
NT = (((1,), (1,)), ((), ()))

V_CHUNKS = (0, 8, 16)
W4_CHUNKS = (0, 48, 80, 96)
NV = len(V_CHUNKS) - 1
NW4 = len(W4_CHUNKS) - 1

AG = 4
T0 = 15
STEP = 6.2
PUSH = 1.0
XPOSE = 2.0
LAT = 170
REV_UNTIL = 240
REV_PER = 2
ORDER_LAYER1 = ("z", "k")
ORDER_LAYER2 = ("z", "k0", "w", "k1", "q")


def _tiles_cache(c):
    t = jnp.transpose(c[0], (0, 2, 1)).reshape(NP, 24, 2, 8, SK // 128, 128)
    return jnp.transpose(t, (0, 1, 2, 4, 3, 5))


def _tiles_weight(w):
    k, n = w.shape
    return jnp.transpose(w.reshape(k // 16, 2, 8, n // 128, 128), (0, 1, 3, 2, 4))


def _as_bf16(words):
    n = words.shape[0]
    return pltpu.bitcast(words.reshape(n * 8, 128), jnp.bfloat16)


def _mm(a, b):
    return jnp.dot(a, b, preferred_element_type=jnp.float32)


def _layernorm(x):
    m = jnp.mean(x, axis=-1, keepdims=True)
    d = x - m
    v = jnp.mean(d * d, axis=-1, keepdims=True)
    return d * lax.rsqrt(v + EPS)


def _ln_stats(x):
    m = jnp.mean(x, axis=-1, keepdims=True)
    d = x - m
    s1 = jnp.mean(d, axis=-1, keepdims=True)
    s2 = jnp.mean(d * d, axis=-1, keepdims=True)
    r = lax.rsqrt(s2 + EPS)
    r2 = lax.rsqrt(r * r * (s2 - s1 * s1) + EPS)
    return m, s1, r, r2


def _gelu(x):
    c = np.float32(0.7978845608028654)
    return 0.5 * x * (1.0 + jnp.tanh(c * (x + np.float32(0.044715) * (x * x * x))))


def _lhs_tiles(x):
    return [x[:, 128 * k:128 * k + 128].astype(jnp.bfloat16) for k in range(ND)]


def _kernel(x_hbm, k_hbm, v_hbm, wq_hbm, wo_hbm, w3_hbm, w4_hbm, o_ref,
            xbuf, kbuf, vbuf, wqbuf, wobuf, w3buf, w4buf,
            lbuf, pbuf, zbuf, ibuf, mlbuf, obuf, ybuf, sbuf, xacc_buf, csbuf, sems):
    ki = k_hbm.bitcast(jnp.int32)
    vi = v_hbm.bitcast(jnp.int32)

    def kv_copy(t, i, b):
        src, dst, ch = ((ki, kbuf, (0, NP)), (vi, vbuf, V_CHUNKS))[t]
        g0, n = ch[i], ch[i + 1] - ch[i]
        return pltpu.make_async_copy(src.at[pl.ds(g0, n), :, b, pl.ds(CB0, NCB)],
                                     dst.at[pl.ds(g0, n), :, :, pl.ds(4 * b, 4), :],
                                     sems.at[0 if t == 0 else i])

    def w_copy(i, b, part=None):
        src, dst = ((wq_hbm, wqbuf), (wo_hbm, wobuf), (w3_hbm, w3buf), (w4_hbm, w4buf))[i]
        src = src.bitcast(jnp.int32)
        if part is None:
            return pltpu.make_async_copy(src.at[:, b], dst.at[:, :, pl.ds(4 * b, 4), :],
                                         sems.at[0 if i == 0 else NV + i - 1])
        a0, n = W4_CHUNKS[part], W4_CHUNKS[part + 1] - W4_CHUNKS[part]
        return pltpu.make_async_copy(src.at[pl.ds(a0, n), b],
                                     dst.at[pl.ds(a0, n), :, pl.ds(4 * b, 4), :],
                                     sems.at[NV + 2 + part])

    x_copy = pltpu.make_async_copy(x_hbm, xbuf, sems.at[0])
    x_copy.start()
    for b in range(2):
        w_copy(0, b).start()
    for t, i in [(0, 0)] + [(1, i) for i in range(NV)]:
        for b in range(2):
            kv_copy(t, i, b).start()
    for i in (1, 2):
        for b in range(2):
            w_copy(i, b).start()
    for part in range(NW4):
        for b in range(2):
            w_copy(3, b, part).start()

    def wait_w(i, part=None):
        for b in range(2):
            w_copy(i, b, part).wait()

    def wait_kv(t, i):
        for b in range(2):
            kv_copy(t, i, b).wait()

    rows = lax.broadcasted_iota(jnp.int32, (8, 128), 0)
    lanes = lax.broadcasted_iota(jnp.int32, (8, 128), 1)
    lane_lo = lanes < 64

    def mm_tiles(lhs, rhs_words, tie=None):
        tot = None
        for t, l in enumerate(lhs):
            w = [rhs_words[8 * t + i] for i in range(8)]
            if tie is not None:
                w[0] = tie(w[0])
            r = _mm(l, pltpu.bitcast(jnp.concatenate(w, axis=0), jnp.bfloat16))
            tot = r if tot is None else tot + r
        return tot

    def store_L(g, q):
        for r in range(4):
            ra = rows == 2 * r
            rb = rows == 2 * r + 1
            lbuf[g, r, 0] = jnp.where(ra, q[0], 0.0).astype(jnp.bfloat16)
            lbuf[g, r, 1] = jnp.where((ra & lane_lo) | (rb & (~lane_lo)), q[1], 0.0).astype(jnp.bfloat16)
            lbuf[g, r, 2] = jnp.where(rb, q[2], 0.0).astype(jnp.bfloat16)

    def store_y(y):
        for k, t in enumerate(_lhs_tiles(y)):
            ybuf[k] = t

    def q_tile(g, c, tie=None):
        return mm_tiles([ybuf[k] for k in range(ND)], wqbuf[:, 3 * g + c], tie) * QSCALE

    def make_q(g):
        store_L(g, [q_tile(g, c) for c in range(3)])

    def qk_block(g, cb, tie=None):
        return mm_tiles([lbuf[g, cb % 4, t] for t in range(3)], kbuf[g, :, cb], tie)

    def qk_all(g):
        out = []
        for i in range(8):
            tot = None
            for r in range(4):
                s = qk_block(g, 4 * i + r)
                tot = s if tot is None else tot + s
            out.append(tot)
        return out

    def softmax_to(slot, g, sc, m=None):
        if sc is None:
            sc = [sbuf[i] for i in range(8)]
        else:
            m = sc[0]
            for s in sc[1:]:
                m = jnp.maximum(m, s)
        m = jnp.maximum(m, pltpu.roll(m, 2, 0))
        m = jnp.maximum(m, pltpu.roll(m, 4, 0))
        tot = None
        for i in range(8):
            p = jnp.exp2(sc[i] - m)
            pbuf[slot, 8 * i:8 * i + 8, :] = p
            tot = p if tot is None else tot + p
        tot = tot + pltpu.roll(tot, 2, 0)
        tot = tot + pltpu.roll(tot, 4, 0)
        mlbuf[g, 0] = m
        mlbuf[g, 1] = tot

    def lane_weights(g, slot):
        m = mlbuf[g, 0]
        M = jnp.max(m, axis=1, keepdims=True)
        c = jnp.exp2(m - M)
        L = jnp.sum(c * mlbuf[g, 1], axis=1, keepdims=True)
        ibuf[slot, 0:8, :] = c / L

    def pv_steps(g, slot, zslot):
        for e in range(2):
            for a0 in range(0, 12, AG):
                acc = [None] * AG
                for cb in range(NCB):
                    row = 8 * (cb // 4) + 2 * (cb % 4) + e
                    p = pbuf[slot, pl.ds(row, 8, stride=0), :]
                    hook = yield acc
                    p = hook(p)
                    p = jnp.concatenate([p, p], axis=0)
                    for a in range(AG):
                        w = vbuf[g, 12 * e + a0 + a, cb]
                        t = pltpu.bitcast(w, jnp.bfloat16).astype(jnp.float32) * p
                        acc[a] = t if acc[a] is None else acc[a] + t
                for a in range(AG):
                    zbuf[zslot, pl.ds(16 * (12 * e + a0 + a), 16), :] = acc[a]
        yield None

    def o_rows(zslot, tie=None):
        wa = ibuf[zslot, pl.ds(0, 8, stride=0), :]
        wb = ibuf[zslot, pl.ds(1, 8, stride=0), :]
        lw = [wa.astype(jnp.bfloat16), jnp.where(rows < 4, wa, wb).astype(jnp.bfloat16),
              wb.astype(jnp.bfloat16)]
        o = []
        for t in range(3):
            z = zbuf[zslot, pl.ds(128 * t, 128), :]
            if tie is not None:
                z0 = pltpu.bitcast(tie(pltpu.bitcast(z[0:8], jnp.int32)), jnp.float32)
                z = jnp.concatenate([z0, z[8:]], axis=0)
            z = z.astype(jnp.bfloat16)
            o.append(lax.dot_general(lw[t], z, NT, preferred_element_type=jnp.float32))
        o[1] = jnp.where((rows < 4) == lane_lo, o[1], pltpu.roll(o[1], 4, 0))
        return o

    def store_o(slot, o):
        for t in range(3):
            obuf[slot, t] = o[t].astype(jnp.bfloat16)

    def wo_tile(slot, g, c):
        return mm_tiles([obuf[slot, t] for t in range(3)], wobuf[pl.ds(24 * g, 24), c])

    x_copy.wait()
    wait_w(0)
    wait_kv(0, 0)
    wait_kv(1, 0)
    x = jnp.broadcast_to(xbuf[0].astype(jnp.float32), (8, D))
    pbuf[:, 64:72, :] = jnp.zeros((2, 8, 128), jnp.float32)
    ibuf[0] = jnp.zeros((16, 128), jnp.float32)
    ibuf[:, 8:16, :] = jnp.zeros((NP + 1, 8, 128), jnp.float32)
    zbuf[0] = jnp.zeros((384, 128), jnp.float32)
    zero = jnp.zeros((8, 128), jnp.float32)

    def body(g, order):
        slot = g & 1
        gn = jnp.minimum(g + 1, NP - 1)
        gq = jnp.minimum(g + 2, NP - 1)
        gp = jnp.maximum(g - 1, 0)
        true = pbuf[0, 64:72, :] == 0.0
        lane_weights(g, g + 1)
        st = {"sc": [None] * 8, "q": [None] * 3, "m": None}

        def mk_tie(av):
            if av is None:
                return None

            def tie(w):
                for _ in range(REV_PER):
                    flat, rot = av
                    w = jnp.where(true, w, pltpu.bitcast(flat[rot[0] % len(flat)], jnp.int32))
                    rot[0] += 1
                return w
            return tie

        def t_q(c):
            def fn(av):
                r = q_tile(gq, c, mk_tie(av))
                st["q"][c] = r
                if c == 2:
                    store_L(gq, st["q"])
                return r
            return (40, fn)

        def t_z():
            def fn(av):
                o = o_rows(g, mk_tie(av))
                store_o(g, o)
                return o[2]
            return (24 * XPOSE, fn)

        def t_w(c):
            def fn(av):
                r = xacc_buf[c] + wo_tile(g, gp, c)
                xacc_buf[c] = r
                return r
            return (24, fn)

        def t_k(cb):
            def fn(av):
                i, r = divmod(cb, 4)
                s = qk_block(gn, cb, mk_tie(av))
                st["sc"][i] = s if r == 0 else st["sc"][i] + s
                if r == 3:
                    sbuf[i] = st["sc"][i]
                    st["m"] = st["sc"][i] if st["m"] is None else jnp.maximum(st["m"], st["sc"][i])
                    return st["m"]
                return st["sc"][i]
            return (24, fn)

        groups = {"q": lambda: [t_q(c) for c in range(3)], "z": lambda: [t_z()],
                  "w": lambda: [t_w(c) for c in range(ND)],
                  "k0": lambda: [t_k(cb) for cb in range(16)],
                  "k1": lambda: [t_k(cb) for cb in range(16, 32)],
                  "k": lambda: [t_k(cb) for cb in range(32)]}
        tasks = [t for name in order for t in groups[name]()]
        issue, t = [], T0
        for n, _ in tasks:
            t += n * PUSH
            issue.append(t)

        gen = pv_steps(g, slot, g + 1)
        acc = next(gen)
        nsteps = 64 * (12 // AG)
        step, nxt, pending, last_acc, rot = 0, 0, [], None, [0]
        while acc is not None:
            now = T0 + STEP * step
            last = step == nsteps - 1
            if acc[0] is not None:
                last_acc = ([h for v in acc for h in (v[0:8], v[8:16])], rot)
            while nxt < len(tasks) and (issue[nxt] <= now + STEP or last):
                val = tasks[nxt][1](last_acc if issue[nxt] <= REV_UNTIL else None)
                pending.append((issue[nxt] + LAT, val))
                nxt += 1
            ready = [v for tt, v in pending if tt <= now or last]
            pending = [(tt, v) for tt, v in pending if not (tt <= now or last)]

            def hook(p, ready=ready):
                for v in ready:
                    p = jnp.where(true, p, v)
                return p
            acc = gen.send(hook)
            step += 1
        softmax_to(1 - slot, gn, None, st["m"])

    def attn_first(x):
        store_y(_layernorm(x))
        ones = [jnp.ones((8, 128), jnp.bfloat16)] * ND
        for c in range(6):
            csbuf[c] = mm_tiles(ones, wqbuf[:, c])

        def q_body(g, c):
            make_q(g)
            return c
        lax.fori_loop(0, NP, q_body, 0)
        softmax_to(0, 0, qk_all(0))

        def loop(g, c):
            for i in range(1, NV):
                pl.when(g == V_CHUNKS[i])(functools.partial(wait_kv, 1, i))
            body(g, ORDER_LAYER1)
            return c
        lax.fori_loop(0, NP, loop, 0)
        store_o(NP, o_rows(NP))
        wait_w(1)

        def wo_body(i, xacc):
            xacc = list(xacc)
            for j in range(4):
                g = i * 4 + j
                for c in range(ND):
                    xacc[c] = xacc[c] + wo_tile(g + 1, g, c)
            return tuple(xacc)
        xacc = lax.fori_loop(0, NP // 4, wo_body, (zero,) * ND)
        return x + jnp.concatenate(xacc, axis=1)

    def attn_second(x):
        xb = _lhs_tiles(x)
        raw = [mm_tiles(xb, wqbuf[:, c]) for c in range(6)]
        m, _, r, _ = _ln_stats(x)
        for g in range(2):
            store_L(g, [(raw[c] - m * csbuf[c]) * (r * QSCALE) for c in range(3 * g, 3 * g + 3)])
        store_y((x - m) * r)
        softmax_to(0, 0, qk_all(0))
        for c in range(ND):
            xacc_buf[c] = zero

        def loop(g, c):
            body(g, ORDER_LAYER2)
            return c
        lax.fori_loop(0, NP, loop, 0)
        store_o(NP, o_rows(NP))
        xacc = [xacc_buf[c] + wo_tile(NP, NP - 1, c) for c in range(ND)]
        return x + jnp.concatenate(xacc, axis=1)

    def mlp_layer(x, first):
        m, s1, r, r2 = _ln_stats(x)
        y = (x - m) * r
        if first:
            wait_w(2)
            ub = _lhs_tiles((x - m - s1) * (r * r2))
            h = jnp.concatenate([mm_tiles(ub, w3buf[:, c]) for c in range(NF)], axis=1)
        else:
            xb = _lhs_tiles(x)
            raw = [mm_tiles(xb, w3buf[:, c]) for c in range(NF)]
            h = jnp.concatenate([(raw[c] - (m + s1) * csbuf[6 + c]) * (r * r2) for c in range(NF)],
                                axis=1)
        h_bf = _gelu(h).astype(jnp.bfloat16)
        if first:
            ones = [jnp.ones((8, 128), jnp.bfloat16)] * ND
            for c in range(NF):
                csbuf[6 + c] = mm_tiles(ones, w3buf[:, c])
        h2 = [None] * ND
        chunks = W4_CHUNKS if first else tuple(range(0, FF // 16 + 1, 8))
        for part in range(len(chunks) - 1):
            if first:
                wait_w(3, part)
            a0, a1 = chunks[part], chunks[part + 1]
            for c in range(ND):
                t = _mm(h_bf[:, 16 * a0:16 * a1], _as_bf16(w4buf[a0:a1, c]))
                h2[c] = t if h2[c] is None else h2[c] + t
        return x + (y + jnp.concatenate(h2, axis=1))

    x = attn_first(x)
    x = mlp_layer(x, True)
    x = attn_second(x)
    x = mlp_layer(x, False)
    o_ref[0] = x[0:1, :].astype(o_ref.dtype)


@jax.jit
def pallas_interleave_layers__sliding_block_cached__mixer_s_mlp__decode_kernel(
    A_x: jax.Array,
    A_k_cache: jax.Array,
    A_v_cache: jax.Array,
    A_wq: jax.Array,
    A_wo: jax.Array,
    B_x: jax.Array,
    B_w1: jax.Array,
    B_w2: jax.Array,
    B_w3: jax.Array,
    B_w4: jax.Array,
):
    del B_x, B_w1, B_w2
    return pl.pallas_call(
        _kernel,
        out_shape=jax.ShapeDtypeStruct((1, 1, D), A_x.dtype),
        in_specs=[pl.BlockSpec(memory_space=pl.ANY)] * 7,
        out_specs=pl.BlockSpec(memory_space=pltpu.VMEM),
        scratch_shapes=[
            pltpu.VMEM((1, 1, D), jnp.bfloat16),
            pltpu.VMEM((NP, 24, NCB, 8, 128), jnp.int32),
            pltpu.VMEM((NP, 24, NCB, 8, 128), jnp.int32),
            pltpu.VMEM((D // 16, NH * DH // 128, 8, 128), jnp.int32),
            pltpu.VMEM((NH * DH // 16, ND, 8, 128), jnp.int32),
            pltpu.VMEM((D // 16, NF, 8, 128), jnp.int32),
            pltpu.VMEM((FF // 16, ND, 8, 128), jnp.int32),
            pltpu.VMEM((NP, 4, 3, 8, 128), jnp.bfloat16),
            pltpu.VMEM((2, 72, 128), jnp.float32),
            pltpu.VMEM((NP + 1, 384, 128), jnp.float32),
            pltpu.VMEM((NP + 1, 16, 128), jnp.float32),
            pltpu.VMEM((NP, 2, 8, 128), jnp.float32),
            pltpu.VMEM((NP + 1, 3, 8, 128), jnp.bfloat16),
            pltpu.VMEM((ND, 8, 128), jnp.bfloat16),
            pltpu.VMEM((8, 8, 128), jnp.float32),
            pltpu.VMEM((ND, 8, 128), jnp.float32),
            pltpu.VMEM((6 + NF, 8, 128), jnp.float32),
            pltpu.SemaphoreType.DMA((NV + 2 + NW4,)),
        ],
        compiler_params=pltpu.CompilerParams(vmem_limit_bytes=127 * 1024 * 1024),
    )(A_x, _tiles_cache(A_k_cache), _tiles_cache(A_v_cache), _tiles_weight(A_wq),
      _tiles_weight(A_wo), _tiles_weight(B_w3), _tiles_weight(B_w4))
```
